```python
import os as _os
_os.environ.setdefault("JAX_PLATFORMS", "cpu")
import jax
import jax.numpy as jnp

def _softmax(x, axis=-1):
    return jax.nn.softmax(x, axis=axis)
def _gelu(x):
    return jax.nn.gelu(x, approximate=True)
def _silu(x):
    return jax.nn.silu(x)
def _sigmoid(x):
    return jax.nn.sigmoid(x)
def _layernorm(x, axis=-1, eps=1e-5):
    m = jnp.mean(x, axis=axis, keepdims=True)
    v = jnp.var(x, axis=axis, keepdims=True)
    return (x - m) / jnp.sqrt(v + eps)
def _scatter_add(tgt, idx, src, axis=0):
    return tgt.at[idx].add(src)
def _segment_sum(src, seg, n):
    return jax.ops.segment_sum(src, seg, n)
class _Rng:
    def __init__(self, key):
        self._k = key
    def _next(self):
        self._k, sub = jax.random.split(self._k)
        return sub
    def normal(self, shape):
        return jax.random.normal(self._next(), shape, dtype=jnp.bfloat16)
    def randint(self, lo, hi, shape):
        return jax.random.randint(self._next(), shape, lo, hi, dtype=jnp.int32)
    def uniform(self, shape, lo=0.0, hi=1.0):
        return jax.random.uniform(self._next(), shape, jnp.bfloat16, lo, hi)
    def permutation(self, n):
        return jax.random.permutation(self._next(), n)


kernel_name = 'interleave_layers__linear_attn_block__mha_block__prompt'

def setup_inputs():
    _rng = _Rng(jax.random.key(int.from_bytes(__import__("os").urandom(4), "little")))
    _w = (lambda a: (lambda t: t.astype(jnp.bfloat16) if jnp.issubdtype(t.dtype, jnp.floating) else t)(jnp.asarray(a)))
    def _A_setup():
        B, S, D = 1, 2048, 1024
        return {
            "x": _w((lambda *s: _rng.normal(s) * 0.05)(B, S, D)),
            "wqkv": _w((lambda *s: _rng.normal(s) * 0.1)(D, 3 * D)),
            "wo": _w((lambda *s: _rng.normal(s) * 0.1)(D, D)),
        }
    _A_in = _A_setup()

    def _B_setup():
        B, S, D, H = 1, 2048, 1024, 32
        return {
            "x": _w((lambda *s: _rng.normal(s) * 0.05)(B, S, D)),
            "wqkv": _w((lambda *s: _rng.normal(s) * 0.1)(D, 3 * D)),
            "wo": _w((lambda *s: _rng.normal(s) * 0.05)(D, D)),
        }
    _B_in = _B_setup()

    return {
        "A_x": _A_in["x"],
        "A_wqkv": _A_in["wqkv"],
        "A_wo": _A_in["wo"],
        "B_x": _B_in["x"],
        "B_wqkv": _B_in["wqkv"],
        "B_wo": _B_in["wo"],
    }

def reference(A_x, A_wqkv, A_wo, B_x, B_wqkv, B_wo):
    def _A_ref(x, wqkv, wo):
        B, S, D = x.shape
        H = 32; Dh = D // H
        qkv = (lambda x, *d: x.transpose(*d))((x @ wqkv).reshape(B, S, 3, H, Dh), 2, 0, 3, 1, 4)
        q, k, v = qkv[0], qkv[1], qkv[2]
        phi = lambda t: jnp.where(t > 0, t + 1, jnp.exp(t)) + 1e-6
        pq, pk = phi(q), phi(k)
        kv = jnp.einsum("bhsd,bhse->bhde", pk, v)
        z = jnp.einsum("bhsd->bhd", pk)
        num = jnp.einsum("bhqd,bhde->bhqe", pq, kv)
        den = jnp.einsum("bhqd,bhd->bhq", pq, z)[..., None] + 1e-6
        o = num / den
        return (lambda x, *d: x.transpose(*d))(o, 0, 2, 1, 3).reshape(B, S, D) @ wo

    def _B_ref(x, wqkv, wo):
        B, S, D = x.shape
        H = 32
        Dh = D // H
        qkv = (lambda x, *d: x.transpose(*d))((x @ wqkv).reshape(B, S, 3, H, Dh), 2, 0, 3, 1, 4)
        q, k, v = qkv[0], qkv[1], qkv[2]
        scores = jnp.einsum("bhqd,bhkd->bhqk", q, k) * (Dh ** -0.5)
        p = _softmax(scores, axis=-1)
        o = jnp.einsum("bhqk,bhkd->bhqd", p, v)
        return (lambda x, *d: x.transpose(*d))(o, 0, 2, 1, 3).reshape(B, S, D) @ wo

    x = A_x
    x = x + _A_ref(_layernorm(x, axis=-1), A_wqkv, A_wo)
    x = x + _B_ref(_layernorm(x, axis=-1), B_wqkv, B_wo)
    x = x + _A_ref(_layernorm(x, axis=-1), A_wqkv, A_wo)
    x = x + _B_ref(_layernorm(x, axis=-1), B_wqkv, B_wo)
    return x
```

```python
import functools
import numpy as np
import jax
import jax.numpy as jnp
from jax import lax
import jax.experimental.pallas as pl
import jax.experimental.pallas.tpu as pltpu

S, D, H, DH = 2048, 1024, 32, 32
G = D // 128
F32, BF16, U32 = jnp.float32, jnp.bfloat16, jnp.uint32
QSCALE = float(DH ** -0.5 * np.log2(np.e))


def _dot(a, b):
    return jnp.dot(a, b, preferred_element_type=F32)


def _pk(x):
    return pltpu.bitcast(x.astype(BF16), U32)


def _up(x):
    return pltpu.bitcast(x, BF16)


def _ln(x):
    m = jnp.mean(x, axis=-1, keepdims=True)
    xc = x - m
    v = jnp.mean(xc * xc, axis=-1, keepdims=True)
    return xc * lax.rsqrt(v + 1e-5)


def _phi(t):
    return jnp.where(t > 0, t + 1.0, jnp.exp(t)) + 1e-6


def make(TM=512, NB=512, QB=512, CK=128, LEAD=1, scopes=False, flags=None):
    NT = S // TM
    NQ = S // QB
    NC = S // CK
    scope = jax.named_scope if scopes else (lambda n: _Null())

    def kernel(x_hbm, wa_hbm, woa_hbm, wb_hbm, wob_hbm, out_hbm,
               xin, wa, woa, wb, wob, xres, xn, pq, kvacc, zacc, mmat, zmat, rbuf,
               qt, kk, vt, ob, s0, s1, s2, s3, sem_in, sem_out):
        sbuf = (s0, s1, s2, s3)
        cps = [pltpu.make_async_copy(a, b, sem_in.at[i]) for i, (a, b) in enumerate(
            [(x_hbm, xin), (wa_hbm, wa), (woa_hbm, woa), (wb_hbm, wb), (wob_hbm, wob)])]
        for c in cps:
            c.start()

        def rows(i):
            return pl.ds(pl.multiple_of(i * TM, TM), TM)

        def prow(i):
            return pl.ds(pl.multiple_of(i * (TM // 2), TM // 2), TM // 2)

        def ln_in(i, slot):
            x = xin[rows(i), :].astype(F32)
            xres[rows(i), :] = x
            xn[slot] = _pk(_ln(x))

        def proj_res(i, lhs, w):
            for n in range(D // NB):
                cs = slice(n * NB, (n + 1) * NB)
                xres[rows(i), cs] = xres[rows(i), cs] + _dot(lhs(), w(cs))

        def ln_res(i, slot):
            xn[slot] = _pk(_ln(xres[rows(i), :]))

        def a_qkv(i, slot):
            pks, vs = [], []
            for n in range(D // NB):
                k = _dot(_up(xn[slot]), wa[:, D + n * NB: D + (n + 1) * NB])
                k = _phi(k)
                zacc[:, n * NB:(n + 1) * NB] += jnp.sum(k.reshape(TM // 8, 8, NB), axis=0)
                pks.append(k.astype(BF16))
            for n in range(D // NB):
                v = _dot(_up(xn[slot]), wa[:, 2 * D + n * NB: 2 * D + (n + 1) * NB])
                vs.append(v.astype(BF16))
            for n in range(D // NB):
                q = _dot(_up(xn[slot]), wa[:, n * NB:(n + 1) * NB])
                pq[prow(i), n * NB:(n + 1) * NB] = _pk(_phi(q))
            for g in range(G):
                n, o = divmod(g * 128, NB)
                kvacc[g] += lax.dot_general(pks[n][:, o:o + 128], vs[n][:, o:o + 128],
                                            (((0,), (0,)), ((), ())), preferred_element_type=F32)

        def a_zero():
            kvacc[...] = jnp.zeros(kvacc.shape, F32)
            zacc[...] = jnp.zeros(zacc.shape, F32)

        def a_mid():
            r = lax.broadcasted_iota(jnp.int32, (128, 128), 0) // DH
            c = lax.broadcasted_iota(jnp.int32, (128, 128), 1) // DH
            for g in range(G):
                kv = jnp.where(r == c, kvacc[g], 0.0).astype(BF16)
                mmat[g * 64:(g + 1) * 64, :] = _pk(_dot(kv, woa[g * 128:(g + 1) * 128, :]))
                z = jnp.sum(zacc[:, g * 128:(g + 1) * 128], axis=0, keepdims=True)
                zt = jnp.broadcast_to(z, (128, 128)).T
                zmat[g] = _pk(jnp.where(r == c, zt, 0.0))

        def a_den(i):
            for g in range(G):
                p = _up(pq[prow(i), g * 128:(g + 1) * 128])
                den = _dot(p, _up(zmat[g])) + 1e-6
                rbuf[:, g * 128:(g + 1) * 128] = _pk(p.astype(F32) / den)

        def b_k(i, slot):
            for n in range(D // NB):
                k = _pk(_dot(_up(xn[slot]), wb[:, D + n * NB: D + (n + 1) * NB]))
                for j in range(NB // 128):
                    kk[n * (NB // 128) + j, prow(i), :] = k[:, j * 128:(j + 1) * 128]

        def b_qv(i, slot):
            for n in range(D // NB):
                q = _dot(_up(xn[slot]), wb[:, n * NB:(n + 1) * NB]) * QSCALE
                qt[i, n * (NB // 2):(n + 1) * (NB // 2), :] = _pk(q.T)
            for n in range(D // NB):
                v = _dot(_up(xn[slot]), wb[:, 2 * D + n * NB: 2 * D + (n + 1) * NB])
                vt[i, n * (NB // 2):(n + 1) * (NB // 2), :] = _pk(v.T)

        def attention():
            assert QB == TM
            LAG = NC + LEAD
            NIT = G * NQ

            def a_chunk(it, j, c, m):
                g, qb = it // NQ, it % NQ
                qh = qt[qb, pl.ds(pl.multiple_of(g * 64 + j * 16, 16), 16), :]
                parts = [jnp.zeros((16, QB), U32)] * 4
                parts[j] = qh
                qm = _up(jnp.concatenate(parts, axis=0))
                s = _dot(_up(kk[g, c * (CK // 2):(c + 1) * (CK // 2), :]), qm)
                sbuf[j][c] = s
                mc = jnp.max(s.reshape(CK // 8, 8, QB), axis=0)
                return mc if m is None else jnp.maximum(m, mc)

            def fin_max(m):
                return jnp.broadcast_to(jnp.max(m, axis=0, keepdims=True), (8, QB))

            m_done = m_run = None
            for t in range(LAG):
                j, c = divmod(t, NC)
                m_run = a_chunk(0, j, c, m_run)
                if c == NC - 1:
                    m_done, m_run = fin_max(m_run), None

            def body(it, carry):
                m_cur, m_run = carry
                zero = it // NIT
                nxt = jnp.minimum(it + 1, NIT - 1)
                g, qb = it // NQ, it % NQ
                maxes = {0: m_cur}
                lh, ah, outs = [], [], []
                l = acc = None
                for t in range(4 * NC):
                    u, c = divmod(t + LAG, NC)
                    m_run = a_chunk(it if u < 4 else nxt, u % 4, c, m_run)
                    if c == NC - 1:
                        maxes[u], m_run = fin_max(m_run), None
                    j, c = divmod(t, NC)
                    m = maxes[j]
                    if lh:
                        m = jnp.where(lh[-1] < 0, ah[-2][0:8] if len(ah) > 1 else lh[-1], m)
                    p = jnp.exp2(sbuf[j][c + zero].reshape(CK // 8, 8, QB) - m[None])
                    for r in reversed(range(CK // 16)):
                        lc = p[2 * r] + p[2 * r + 1]
                        l = lc if l is None else l + lc
                    kt, ko = divmod(c * CK, TM)
                    v = _up(vt[kt, pl.ds(pl.multiple_of(g * 64 + j * 16, 16), 16), ko:ko + CK])
                    o = _dot(v, p.reshape(CK, QB).astype(BF16))
                    acc = o if acc is None else acc + o
                    lh.append(l)
                    ah.append(acc)
                    if c == NC - 1:
                        outs.append(acc * (1.0 / jnp.sum(l, axis=0, keepdims=True)))
                        l = acc = None
                ob[g, pl.ds(pl.multiple_of(qb * (QB // 2), QB // 2), QB // 2), :] = _pk(
                    jnp.concatenate(outs, axis=0).T)
                return maxes[4], m_run

            lax.fori_loop(0, NIT, body, (m_done, m_run))

        def o_lhs(i):
            return lambda: _up(jnp.concatenate([ob[g, prow(i), :] for g in range(G)], axis=1))

        def pass_a_in(first):
            def pre(i, slot):
                if first:
                    ln_in(i, slot)
                else:
                    proj_res(i, o_lhs(i), lambda cs: wob[:, cs])
                    ln_res(i, slot)
            a_zero()
            pre(0, 0)

            def body(i, c):
                pre(i + 1, (i + 1) % 2)
                a_qkv(i, i % 2)
                return c
            lax.fori_loop(0, NT - 1, body, 0)
            a_qkv(NT - 1, (NT - 1) % 2)

        def pass_b_in():
            a_den(0)
            proj_res(0, lambda: _up(rbuf[...]), lambda cs: _up(mmat[:, cs]))
            ln_res(0, 0)

            def body(i, c):
                a_den(i + 1)
                b_k(i, i % 2)
                proj_res(i + 1, lambda: _up(rbuf[...]), lambda cs: _up(mmat[:, cs]))
                ln_res(i + 1, (i + 1) % 2)
                b_qv(i, i % 2)
                return c
            lax.fori_loop(0, NT - 1, body, 0)
            b_qv(NT - 1, (NT - 1) % 2)
            b_k(NT - 1, (NT - 1) % 2)

        def out_copy(i):
            return pltpu.make_async_copy(xin.at[rows(i), :], out_hbm.at[rows(i), :], sem_out.at[i])

        def pass_out():
            def body(i, c):
                for n in range(D // NB):
                    cs = slice(n * NB, (n + 1) * NB)
                    xin[rows(i), cs] = (xres[rows(i), cs] + _dot(o_lhs(i)(), wob[:, cs])).astype(BF16)
                out_copy(i).start()
                return c
            lax.fori_loop(0, NT, body, 0)
            for i in range(NT):
                out_copy(i).wait()

        with scope("wait0"):
            cps[0].wait()
            cps[1].wait()
        with scope("a_in0"):
            pass_a_in(True)
        cps[2].wait()
        cps[3].wait()
        cps[4].wait()

        def layer(r, c):
            with scope("a_mid"):
                a_mid()
            with scope("b_in"):
                pass_b_in()
            with scope("att"):
                attention()

            @pl.when(r == 0)
            def _():
                with scope("a_in1"):
                    pass_a_in(False)
            return c
        lax.fori_loop(0, 2, layer, 0)
        with scope("out"):
            pass_out()

    def run(A_x, A_wqkv, A_wo, B_x, B_wqkv, B_wo):
        any_spec = pl.BlockSpec(memory_space=pl.ANY)
        out = pl.pallas_call(
            kernel,
            out_shape=jax.ShapeDtypeStruct((S, D), BF16),
            in_specs=[any_spec] * 5,
            out_specs=any_spec,
            scratch_shapes=[
                pltpu.VMEM((S, D), BF16),
                pltpu.VMEM((D, 3 * D), BF16),
                pltpu.VMEM((D, D), BF16),
                pltpu.VMEM((D, 3 * D), BF16),
                pltpu.VMEM((D, D), BF16),
                pltpu.VMEM((S, D), F32),
                pltpu.VMEM((2, TM // 2, D), U32),
                pltpu.VMEM((S // 2, D), U32),
                pltpu.VMEM((G, 128, 128), F32),
                pltpu.VMEM((8, D), F32),
                pltpu.VMEM((D // 2, D), U32),
                pltpu.VMEM((G, 64, 128), U32),
                pltpu.VMEM((TM // 2, D), U32),
                pltpu.VMEM((NT, D // 2, TM), U32),
                pltpu.VMEM((G, S // 2, 128), U32),
                pltpu.VMEM((NT, D // 2, TM), U32),
                pltpu.VMEM((G, S // 2, 128), U32),
            ] + [pltpu.VMEM((NC, CK, QB), F32)] * 4 + [
                pltpu.SemaphoreType.DMA((5,)),
                pltpu.SemaphoreType.DMA((NT,)),
            ],
            compiler_params=pltpu.CompilerParams(vmem_limit_bytes=110 * 2 ** 20, flags=flags),
            name="fused",
        )(A_x.reshape(S, D), A_wqkv, A_wo, B_wqkv, B_wo)
        return out.reshape(1, S, D)
    return run


class _Null:
    def __enter__(self):
        return None

    def __exit__(self, *a):
        return False


@jax.jit
def pallas_interleave_layers__linear_attn_block__mha_block__prompt_kernel(
    A_x: jax.Array,
    A_wqkv: jax.Array,
    A_wo: jax.Array,
    B_x: jax.Array,
    B_wqkv: jax.Array,
    B_wo: jax.Array,
):
    return make()(A_x, A_wqkv, A_wo, B_x, B_wqkv, B_wo)
```

```python
import numpy as np
import jax
import jax.numpy as jnp
from jax import lax
import jax.experimental.pallas as pl
import jax.experimental.pallas.tpu as pltpu

S, D, H, DH = 2048, 1024, 32, 32
G = D // 128
F32, BF16, U32 = jnp.float32, jnp.bfloat16, jnp.uint32
QSCALE = float(DH ** -0.5 * np.log2(np.e))


def _dot(a, b):
    return jnp.dot(a, b, preferred_element_type=F32)


def _pk(x):
    return pltpu.bitcast(x.astype(BF16), U32)


def _up(x):
    return pltpu.bitcast(x, BF16)


def _phi(t):
    return jnp.where(t > 0, t + 1.0, jnp.exp(t)) + 1e-6


_LHS = (((1, 0, 1), (1, 1, 1)), ((0, 0, 1), (1, 1, 1)), ((1, 1, 1),), ((0, 0, 1), (0, 1, 1)),
        ((0, 1, 1), (1, 1, -1)), ((0, 0, 1),), ((1, 0, 1), (0, 0, -1)))
_RHS = (((0, 0, 1),), ((0, 0, 1), (1, 1, 1)), ((1, 0, 1), (0, 0, -1)), ((1, 1, 1),),
        ((1, 0, 1), (1, 1, 1)), ((0, 1, 1), (1, 1, -1)), ((0, 0, 1), (0, 1, 1)))


def _comb(terms, get):
    out = get(*terms[0][:2])
    for i, j, sign in terms[1:]:
        out = out + get(i, j) if sign > 0 else out - get(i, j)
    return out


def _combos(table, k, load):
    q = [[_comb(table[k], lambda i, j: load(2 * i + a, 2 * j + b)) for b in range(2)] for a in range(2)]
    return [_comb(t, lambda a, b: q[a][b]) for t in table]


def _strassen(prod, levels, emit, put, get, base=0):
    if levels == 0:
        return [lambda: emit(0, 0, prod(base))]
    n, h = 7 ** (levels - 1), 2 ** (levels - 1)

    def step(k):
        def e(i, j, v):
            o = 0 if levels == 1 else 4 + 4 * (2 * i + j)
            if k == 0:
                put(o, v)
            elif k == 1:
                put(o + 1, v)
            elif k == 2:
                m2, m1 = get(o), get(o + 1)
                emit(h + i, j, m2 + v)
                put(o + 2, m1 + v)
            elif k == 3:
                put(o + 3, v)
            elif k == 4:
                emit(i, j, (get(o + 2) + v) - get(o + 3))
            elif k == 5:
                emit(i, h + j, get(o + 3) + v)
                put(o + 2, (get(o + 1) + v) - get(o))
            else:
                emit(h + i, h + j, get(o + 2) + v)
        return e
    out = []
    for k in range(7):
        out += _strassen(prod, levels - 1, step(k), put, get, base + k * n)
    return out


def _swap_blocks(t):
    lane = lax.broadcasted_iota(jnp.int32, t[0].shape, 1)
    for bit, sh in ((1, 8), (2, 16)):
        low = (lane & sh) == 0
        t = [jnp.where(low, t[b], pltpu.roll(t[b | bit], sh, 1)) if not b & bit
             else jnp.where(low, pltpu.roll(t[b ^ bit], 128 - sh, 1), t[b]) for b in range(4)]
    return t


class _Task:
    def __init__(self, run, room=0.0, keys=()):
        self.run, self.room, self.keys = run, room, keys

    def __call__(self):
        self.run()


def _weave(main, side=(), lo=0.0, hi=1.0, ahead=2):
    side = list(side)
    last = {key: n for n, t in enumerate(side) for key in getattr(t, "keys", ())}
    total = sum(t.room for t in main)
    k, seen = 0, 0.0
    for n, t in enumerate(main):
        seen += t.room
        must = max([last.get(key, -1) for u in main[n:n + ahead + 1] for key in u.keys], default=-1)
        while k < len(side) and (k <= must or (lo + (hi - lo) * k / len(side)) * total < seen):
            side[k]()
            k += 1
        t()
    for t in side[k:]:
        t()


def make(TM=512, CK=128, LEAD=1, scopes=False, flags=None, only=None,
         nb=70, na=35, w1=(0.04, 0.97), SR=32, ns=16, lag=3, short=0, due=3, ksp=1, expl=0, qop=False, accm=True, cmax=9, shift=1, f1=0.2, f2=0.75, f3=0.82, lag_b=2, due_b=0, PR=64, opace=True, wpace=True, nq=14, t_op=70, t_tr=4):
    QB, UPI, B, R = TM, 8, 4, 49
    NT = S // TM
    NC = S // CK
    BM, BK = TM // B, D // B
    scope = jax.named_scope if scopes else (lambda n: _Null())
    AQ, AK, AV, AO, BQ, BK_, BV, BO = range(8)

    lag0, due0 = lag, due

    def nonlocal_cfg(a, b):
        nonlocal lag, due
        lag, due = a, b

    def kernel(x_hbm, wa_hbm, woa_hbm, wb_hbm, wob_hbm, out_hbm,
               xin, wa, wq, woa, wb, wob, xres, xl, xr, pq, pkt, vb, kvacc, zacc, zrow,
               qt, kk, vt, ot, mu, rs, rden, acc0, acc1, sem_in, sem_out, *bufs):
        wc, tmp, sbuf = bufs[:8], [], bufs[8:]
        ob = pq
        accb = (acc0, acc1)

        def rows(i, off, n):
            return pl.ds(pl.multiple_of(i * TM + off, n), n)

        def zeros(i):
            never[0] = i >> 20
            return [i >> (8 + k) for k in range(8)]

        ticks, owed = [], []
        never = [None]

        def paced(v, zs):
            if len(ticks) < lag:
                return v
            return jnp.where(jnp.broadcast_to(zs[6], v.shape) != 0, jnp.tile(ticks[-lag], (v.shape[0] // 8, v.shape[1] // 128)), v)

        def w_combo(u, src, rho, k, zs):
            def run():
                def load(a, b):
                    v = src(a * BK + rho * 8, b * BK, zs[k])
                    return paced(v, zs) if wpace and (a // 2, b // 2) == _RHS[k][0][:2] else v
                ts = _combos(_RHS, k, load)
                for r, t in enumerate(ts):
                    wc[u][7 * k + r, pl.ds(pl.multiple_of(rho * 8, 8), 8), :] = t.astype(BF16)
                if due:
                    t = ts[4] + ts[6]
                    owed.append((len(ticks) + due, t[:, :128] + t[:, 128:]))
            return run

        def raw(ref, c0):
            return lambda r, c, z: ref[pl.ds(pl.multiple_of(r + z * 8, 8), 8), c0 + c:c0 + c + BK].astype(F32)

        def x_combo(slot, rho, k, load):
            def run():
                ts = _combos(_LHS, k, load)
                for r, t in enumerate(ts):
                    slot[7 * k + r, rho * 8:rho * 8 + 8, :] = t.astype(BF16)
                if due:
                    t = ts[0] + ts[3]
                    owed.append((len(ticks) + due, t[:, :128] + t[:, 128:]))
            return _Task(run, keys=(('xr' if slot is xr else 'xl', k),))

        def by_k(combo, ks):
            return [combo(rho, k) for k in ks for rho in range(BM // 8)]

        def ln_tasks(i, first, zs):
            def ld(r0, n, z, cs=slice(None)):
                if first:
                    return xin[rows(i + z, r0, n), cs].astype(F32)
                return xres[rows(i + z, r0, n), cs]

            def mean(r0):
                def run():
                    x = ld(r0, SR, 0)
                    t = paced(x[:, :128], zs)
                    for g in range(1, G):
                        t = t + x[:, g * 128:(g + 1) * 128]
                    mu[0, r0:r0 + SR, :] = jnp.broadcast_to(jnp.sum(t, axis=-1, keepdims=True) * (1.0 / D), (SR, 128))
                return run

            def rstd(r0):
                def run():
                    x = ld(r0, SR, zs[7]) - jnp.tile(paced(mu[zs[7], r0:r0 + SR, :], zs), (1, G))
                    rs[0, r0:r0 + SR, :] = jnp.broadcast_to(
                        lax.rsqrt(jnp.mean(x * x, axis=-1, keepdims=True) + 1e-5), (SR, 128))
                return run

            def combo(rho, k):
                def load(a, b):
                    r0 = a * BM + rho * 8
                    x = ld(r0, 8, zs[k], slice(b * BK, (b + 1) * BK)) - jnp.tile(paced(mu[zs[k], r0:r0 + 8, :], zs), (1, 2))
                    return x * jnp.tile(rs[zs[k], r0:r0 + 8, :], (1, 2))
                return x_combo(xl, rho, k, load)
            return (lambda lo, hi: [f(r0) for f in (mean, rstd) for r0 in range(lo, hi, SR)]), combo

        def ln_head(main, i, first, zs, lo=2):
            stats, combo = ln_tasks(i, first, zs)
            st = stats(0, TM)
            n1, n2 = int(f1 * len(main)), int(f2 * len(main))
            _weave(main[:n1], st[:TM // SR], lo / n1, 1.0)
            _weave(main[n1:n2], st[TM // SR:], 0.05, 1.0)
            _weave(main[n2:], by_k(combo, range(ksp)), 3 / (len(main) - n2), 0.93)

        def ln_rest(main, i, first, zs):
            _weave(main, by_k(ln_tasks(i, first, zs)[1], range(ksp, 7)), 0.0, f3)

        def o_combos(i, dst, zs):
            def combo(rho, k):
                def load(a, b):
                    v = ob[b + zs[k], rows(i, a * BM + rho * 8, 8), :].astype(F32)
                    return paced(v, zs) if opace and (a // 2, b // 2) == _LHS[k][0][:2] else v
                return x_combo(dst, rho, k, load)
            return by_k(combo, range(7))

        def r_weave(main, i, zs, hi):
            def stats(r0):
                def run():
                    t = [pq[b, rows(i, r0, SR), :].astype(F32).reshape(SR // 8, 8, BK) * paced(zrow[b + zs[7]], zs)[None]
                         for b in range(B)]
                    t = ((t[0] + t[1]) + (t[2] + t[3])).reshape(SR, BK)
                    v = jnp.concatenate([t[:, :128], t[:, 128:]], axis=0)
                    lane = lax.broadcasted_iota(jnp.int32, v.shape, 1)
                    for sh in (1, 2, 4):
                        v = v + jnp.where((lane & sh) != 0, pltpu.roll(v, sh, 1), pltpu.roll(v, 128 - sh, 1))
                    v = pltpu.reciprocal(v + 1e-6, full_range=False)
                    rden[0, r0:r0 + SR, :] = jnp.concatenate([v[:SR], v[SR:]], axis=1)
                return run

            def combo(rho, k):
                def load(a, b):
                    r0 = a * BM + rho * 8
                    return pq[b + zs[k], rows(i, r0, 8), :].astype(F32) * paced(rden[zs[k], r0:r0 + 8, :], zs)
                return x_combo(xr, rho, k, load)
            _weave(main[:ns + 5], [stats(r0) for r0 in range(0, TM, SR)], 0.0, ns / (ns + 5))
            _weave(main[ns + 5:], by_k(combo, range(7)), 0.0, hi)

        def permute_wq(n, zs):
            def run():
                rr, j = slice(n // 2 * PR, n // 2 * PR + PR), n % 2
                cs = [slice(b * BK + j * 128, b * BK + j * 128 + 128) for b in range(B)]
                t = _swap_blocks([paced(pltpu.bitcast(wa[rr, c], F32), zs) for c in cs])
                for b in range(B):
                    wq[rr, cs[b]] = _up(t[b])
            return run

        def burst(dst, table, load, lo, hi, unroll=4):
            def body(n):
                for h in range(unroll):
                    r0 = lo + (n * unroll + h) * 8
                    blk = [[load(a, b, r0) for b in range(B)] for a in range(B)]
                    for k in range(7):
                        for r, t in enumerate(_combos(table, k, lambda a, b: blk[a][b])):
                            dst[7 * k + r, pl.ds(pl.multiple_of(r0, 8), 8), :] = t.astype(BF16)
            loop((hi - lo) // (8 * unroll), body)

        def w_burst(u, ref, c0, lo=0, hi=BK):
            burst(wc[u], _RHS, lambda a, b, r0: raw(ref, c0)(a * BK + r0, b * BK, 0), lo, hi)

        def mm(slot, u, emit, epi):
            def prod(r):
                w = wc[u][r]
                if owed and owed[0][0] <= len(ticks):
                    w = pltpu.bitcast(w, U32)
                    top = w[0:8, 0:128]
                    while owed and owed[0][0] <= len(ticks):
                        top = jnp.where(jnp.broadcast_to(never[0], (8, 128)) != 0,
                                        pltpu.bitcast(owed.pop(0)[1], U32), top)
                    w = _up(jnp.concatenate([jnp.concatenate([top, w[0:8, 128:]], axis=1), w[8:]], axis=0))
                v = _dot(slot[r], w)
                ticks.append(v[0:8, 0:128])
                return v
            adds = (0, 0, 2, 0, 2, 3, 1)
            bank = tmp[20:] if slot is xr else tmp
            held = {}

            def put(n, v):
                if expl >> (n >= 4) & 1:
                    bank[n][0] = v
                else:
                    held[n] = v

            def get(n):
                return bank[n][never[0] >> (len(ticks) % 2)] if expl >> (n >= 4) & 1 else held[n]

            def room(r):
                ko, ki = divmod(max(r - shift, 0), 7)
                return max(cmax - adds[ki] - (adds[ko] + epi if adds[ki] and adds[ko] else 0), 0.5)
            return [_Task(t, room(r), (('xr' if slot is xr else 'xl', r // 7), (u, r // 7))) for r, t in enumerate(_strassen(prod, 2, emit, put, get))]

        def res_proj(i, slot, u, first=False):
            def emit(bi, bj, v):
                rr, cs = rows(i, bi * BM, BM), slice(bj * BK, (bj + 1) * BK)
                xres[rr, cs] = (xin[rr, cs].astype(F32) if first else xres[rr, cs]) + v
            return mm(slot, u, emit, 2)

        def out_copy(i, qi, qj):
            rr, cs = rows(i, qi * (TM // 2), TM // 2), slice(qj * (D // 2), (qj + 1) * (D // 2))
            return pltpu.make_async_copy(xin.at[rr, cs], out_hbm.at[rr, cs], sem_out.at[i * 4 + qi * 2 + qj])

        def out_proj(i, slot):
            def emit(bi, bj, v):
                rr, cs = rows(i, bi * BM, BM), slice(bj * BK, (bj + 1) * BK)
                xin[rr, cs] = (xres[rr, cs] + v).astype(BF16)
                if bi % 2 and bj % 2:
                    out_copy(i, bi // 2, bj // 2).start()
            return mm(slot, BO, emit, 2)

        def a_qkv(i, slot, z=0):
            def emit_k(bi, bj, v):
                v = _phi(v)
                zacc[:, bj * BK:(bj + 1) * BK] += jnp.sum(v.reshape(BM // 8, 8, BK), axis=0)
                pkt[bj * (BK // 2):(bj + 1) * (BK // 2), bi * BM:(bi + 1) * BM] = pltpu.bitcast(v.astype(BF16).T, U32)

            def emit_v(bi, bj, v):
                vb[bi * BM:(bi + 1) * BM, bj * BK:(bj + 1) * BK] = v.astype(BF16)

            def emit_q(bi, bj, v):
                pq[bj, rows(i, bi * BM, BM), :] = _phi(v).astype(BF16)

            def kv(g):
                def run():
                    kvacc[g] += _dot(_up(pkt[g * 64:(g + 1) * 64, :]), vb[:, g * 128:(g + 1) * 128])
                return run
            return (mm(slot, AK, emit_k, 8), mm(slot, AV, emit_v, 1), mm(slot, AQ, emit_q, 7),
                    [_Task(kv(g), cmax - 1) for g in range(G)])

        def b_qkv(i, slot, z=0):
            def transposed(ref, scale):
                def emit(bi, bj, v):
                    v = v if scale is None else v * scale
                    ref[i, bj * (BK // 2):(bj + 1) * (BK // 2), bi * BM:(bi + 1) * BM] = pltpu.bitcast(
                        v.astype(BF16).T, U32)
                return emit

            def emit_k(bi, bj, v):
                v = _pk(v)
                rr = pl.ds(pl.multiple_of(i * (TM // 2) + bi * (BM // 2), BM // 2), BM // 2)
                for j in range(BK // 128):
                    kk[bj * (BK // 128) + j, rr, :] = v[:, j * 128:(j + 1) * 128]
            return (mm(slot, BQ, transposed(qt, QSCALE), 2) + mm(slot, BV, transposed(vt, None), 1)
                    + mm(slot, BK_, emit_k, 2))

        def a_zero():
            kvacc[...] = jnp.zeros(kvacc.shape, F32)
            zacc[...] = jnp.zeros(zacc.shape, F32)

        def a_z():
            for j in range(BK // 128):
                t = _swap_blocks([jnp.broadcast_to(jnp.sum(
                    zacc[:, b * BK + j * 128:b * BK + j * 128 + 128], axis=0, keepdims=True), (8, 128))
                    for b in range(B)])
                for b in range(B):
                    zrow[b, :, j * 128:(j + 1) * 128] = t[b]

        def a_m():
            def piece(g, n):
                def run():
                    same = (lax.broadcasted_iota(jnp.int32, (128, 128), 0) // DH
                            == lax.broadcasted_iota(jnp.int32, (128, 128), 1) // DH)
                    kv = jnp.where(same, kvacc[g], 0.0).astype(BF16)
                    m = _dot(kv, woa[g * 128:(g + 1) * 128, n * 512:(n + 1) * 512])
                    hb, j = divmod(g, 2)
                    for hl in range(4):
                        for dd in range(4):
                            r0 = hl * 32 + hb * 8
                            sbuf[(dd * 2 + j) * 2 + n][0, r0:r0 + 8, :] = m[hl * 32 + dd * 8:hl * 32 + dd * 8 + 8]
                return run
            return [_Task(piece(g, n), cmax - 1) for n in range(2) for g in range(G)]

        def m_src(r0, c0, z):
            return sbuf[(r0 // 128) * 2 + c0 // 512][z, r0 % 128:r0 % 128 + 8, c0 % 512:c0 % 512 + BK]

        def w_all(u, src, k, zs):
            return [w_combo(u, src, rho, k, zs) for rho in range(BK // 8)]

        def attention(final):
            LAG = NC + LEAD
            NS = H * (S // QB) // UPI

            def where(step, u):
                it = 2 * step + u // 4
                return it // G, it % G, u % 4

            def a_chunk(step, u, c, m, z=0):
                qb, g, j = where(step, u)
                parts = [jnp.zeros((16, QB), U32)] * 4
                parts[j] = qt[qb + z, pl.ds(pl.multiple_of(g * 64 + j * 16, 16), 16), :]
                s = _dot(_up(kk[g, c * (CK // 2):(c + 1) * (CK // 2), :]), _up(jnp.concatenate(parts, axis=0)))
                sbuf[(u % 2) * NC + c][0] = s
                mc = jnp.max(s.reshape(CK // 8, 8, QB), axis=0)
                return mc if m is None else jnp.maximum(m, mc)

            def fin_max(m):
                return jnp.broadcast_to(jnp.max(m, axis=0, keepdims=True), (8, QB))

            def flush(step, n):
                qb, g, _ = where(step, 0)
                ob[g // 2, pl.ds(pl.multiple_of(qb * QB + n * 128, 128), 128), :] = (
                    ot[:, n * 128:(n + 1) * 128].astype(BF16).T)

            ot[...] = jnp.zeros(ot.shape, F32)
            m_done = m_run = None
            for t in range(LAG):
                u, c = divmod(t, NC)
                m_run = a_chunk(0, u, c, m_run)
                if c == NC - 1:
                    m_done, m_run = fin_max(m_run), None

            def block(step, m_cur, m_run, zero, extra=None):
                maxes = {0: m_cur}
                lh, ah = [], []
                ticks.clear(), owed.clear()
                l = acc = None
                for t in range(UPI * NC):
                    u, c = divmod(t, NC)
                    qb, g, j = where(step, u)
                    s = sbuf[(u % 2) * NC + c][zero]
                    ua, ca = divmod(t + LAG, NC)
                    more = extra is None or ua < UPI
                    if more:
                        m_run = a_chunk(step, ua, ca, m_run, (zero >> ca) if qop else 0)
                        if ca == NC - 1:
                            maxes[ua], m_run = fin_max(m_run), None
                    if t_tr <= t < t_tr + 2 * (QB // 128) and (t - t_tr) % 2 == 0:
                        flush(jnp.maximum(step - 1, 0), (t - t_tr) // 2)
                    if extra is not None:
                        extra(t)
                    m = maxes[u]
                    if lh:
                        m = jnp.where(lh[-1] < 0, ah[-2][0:8] if len(ah) > 1 and (more or final) else lh[-1], m)
                    p = jnp.exp2(s.reshape(CK // 8, 8, QB) - m[None])
                    for r in reversed(range(CK // 16)):
                        lc = p[2 * r] + p[2 * r + 1]
                        l = lc if l is None else l + lc
                    kt, ko = divmod(c * CK, TM)
                    v = _up(vt[kt, pl.ds(pl.multiple_of(g * 64 + j * 16, 16), 16), ko:ko + CK])
                    o = _dot(v, p.reshape(CK, QB).astype(BF16))
                    if accm:
                        acc = o if acc is None else accb[c % 2][zero] + o
                        if c < NC - 1:
                            accb[(c + 1) % 2][0] = acc
                    else:
                        acc = o if acc is None else acc + o
                    lh.append(l)
                    ah.append(acc)
                    ticks.append(acc[0:8, 0:128])
                    if c == NC - 1:
                        ot[u * DH:(u + 1) * DH, :] = acc * pltpu.reciprocal(
                            jnp.sum(l, axis=0, keepdims=True), full_range=False)
                        l = acc = None
                return maxes.get(UPI), m_run

            m_cur, m_run, z = lax.fori_loop(
                0, NS - 1, lambda i, c: block(i, c[0], c[1], i // NS) + (i // NS,), (m_done, m_run, 0))
            zs = zeros(z)
            T = UPI * NC
            side = o_combos(0, xr, zs)
            if final:
                main = out_proj(0, xr)

                def extra(t):
                    if t >= T - LAG:
                        main.pop(0).run()
                    for _ in range(2 if t > 16 else 0):
                        if side:
                            side.pop(0)()
            else:
                main = res_proj(0, xr, BO)
                stats, combo = ln_tasks(0, False, zs)
                ln = stats(0, TM) + [lambda: None] * 3 + by_k(combo, range(ksp))

                def extra(t):
                    if t == t_op:
                        _weave(main, side, 0.0, 0.8)
                    if 12 < t < t_op:
                        side.pop(0)()
                    if t > t_op + 1 and ln:
                        ln.pop(0)()
            block(NS - 1, m_cur, m_run, z, extra)
            for n in range(QB // 128):
                flush(NS - 1, n)
            return main, zs

        def loop(n, fn):
            def body(i, c):
                ticks.clear(), owed.clear()
                fn(i)
                ticks.clear(), owed.clear()
                return i // n
            return zeros(lax.fori_loop(0, n, body, 0))

        def a_last(first, zs, side):
            k, v, q, kv = a_qkv(NT - 1, xl)
            ln_rest(k, NT - 1, first, zs)
            _weave(v[:2])
            a_z()
            r_weave(v[2:] + q[:2] + kv + q[2:4] + a_m(), 0, zs, 0.98)
            rp = res_proj(0, xr, AO, first)
            _weave(q[4:nq], w_all(AO, m_src, 0, zs) + w_all(AO, m_src, 1, zs), 0.1, 0.9)
            for n in range(7):
                _weave(rp[7 * n:7 * n + 7], w_all(AO, m_src, n + 2, zs) if n < 5 else [])
            ln_head(q[nq:], 0, False, zs)

        def pass_a_in():
            def tile(i):
                zs = zeros(i)
                k, v, q, kv = a_qkv(i, xl)
                ln_rest(k, i, False, zs)
                _weave(v + res_proj(i + 1, xr, BO), o_combos(i + 1, xr, zs), 0.0, 0.9)
                ln_head(q + kv, i + 1, False, zs)
            a_zero()
            if short == 1:
                return loop(NT - 1, tile)
            if short == 2:
                return a_last(False, loop(NT - 1, lambda i: None), [])
            a_last(False, loop(NT - 1, tile), [])

        def pass_b_in(first):
            nonlocal_cfg(lag_b, due_b)
            def tile(i):
                zs = zeros(i)
                main = b_qkv(i, xl)
                ln_rest(main[:R], i, False, zs)
                r_weave(main[R:2 * R] + res_proj(i + 1, xr, AO, first), i + 1, zs, 0.88)
                ln_head(main[2 * R:], i + 1, False, zs)
            zs = loop(NT - 1, tile)
            if short:
                return
            nonlocal_cfg(lag0, due0)
            main = b_qkv(NT - 1, xl, zs[0])
            ln_rest(main[:R], NT - 1, False, zs)
            _weave(main[R:], [t for k in range(7) for t in w_all(BO, raw(wob, 0), k, zs)] if first else [], 0.0, 0.97)

        def pass_out(rest, zs):
            for i in range(NT):
                main = rest if i == 0 else out_proj(i, (xr, xl)[i % 2])
                _weave(main, o_combos(i + 1, (xl, xr)[i % 2], zs) if i + 1 < NT else [], 0.0, 0.97)
            for i in range(NT):
                for q in range(4):
                    out_copy(i, q // 2, q % 2).wait()

        def pass_first():
            jobs = [(x_hbm, xin, 0, TM // 2, 0, D), (x_hbm, xin, TM // 2, TM // 2, 0, D)]
            jobs += [(wa_hbm, wa, a * BK + h * (BK // 2), BK // 2, D, D) for h in range(2) for a in range(B)]
            jobs += [(wa_hbm, wa, 0, D, 2 * D, D), (wa_hbm, wa, 0, D, 0, D), (x_hbm, xin, TM, TM, 0, D),
                     (x_hbm, xin, 2 * TM, S - 2 * TM, 0, D),
                     (wb_hbm, wb, 0, D, 0, 3 * D), (woa_hbm, woa, 0, D, 0, D), (wob_hbm, wob, 0, D, 0, D)]
            cps = [pltpu.make_async_copy(a.at[r:r + nr, c:c + nc], b.at[r:r + nr, c:c + nc], sem_in.at[n])
                   for n, (a, b, r, nr, c, nc) in enumerate(jobs)]
            for c in cps[:10]:
                c.start()
            a_zero()
            stats = ln_tasks(0, True, loop(2, lambda i: None))[0]
            with scope("p_x"):
                for n in range(2):
                    cps[n].wait()
                    _weave([], stats(n * TM // 2, (n + 1) * TM // 2))

                def normed(a, b, r0):
                    rr = pl.ds(pl.multiple_of(a * BM + r0, 8), 8)
                    return ((xin[rr, b * BK:(b + 1) * BK].astype(F32) - jnp.tile(mu[0, rr, :], (1, 2)))
                            * jnp.tile(rs[0, rr, :], (1, 2)))
                burst(xl, _LHS, normed, 0, BM, 1)
            with scope("p_wk"):
                for h in range(2):
                    for c in cps[2 + 4 * h:6 + 4 * h]:
                        c.wait()
                    if h == 1:
                        cps[10].start()
                        cps[11].start()
                    w_burst(AK, wa, D, h * (BK // 2), (h + 1) * (BK // 2))

            def tile(i):
                zs = zeros(i)
                k, v, q, kv = a_qkv(i, xl)
                with scope('tk'):
                    ln_rest(k, i, True, zs)

                @pl.when(i == 0)
                def _():
                    with scope("p_wv"):
                        cps[10].wait()
                        w_burst(AV, wa, 2 * D)
                        cps[11].wait()
                        cps[12].start()
                ticks.clear(), owed.clear(), zeros(i)
                with scope('tv'):
                    _weave(v, [permute_wq(n, zs) for n in range(2 * D // PR)], 0.0, 0.9)

                @pl.when(i == 0)
                def _():
                    with scope("p_wq"):
                        cps[12].wait()
                        for c in cps[13:]:
                            c.start()
                        w_burst(AQ, wq, 0)

                @pl.when(i == 1)
                def _():
                    cps[13].wait()
                ticks.clear(), owed.clear(), zeros(i)
                with scope('tq'):
                    ln_head(q + kv, i + 1, True, zs, 0)
            zs = loop(NT - 1, tile)
            with scope("p_wb"):
                for c in cps[14:]:
                    c.wait()
                for u in (BQ, BK_, BV):
                    w_burst(u, wb, (u - BQ) * D)
            if short == 1:
                return
            a_last(True, loop(2, lambda i: None), [])

        if only:
            {"b_in0": lambda: pass_b_in(True), "b_in1": lambda: pass_b_in(False),
             "att0": lambda: attention(False), "att1": lambda: pass_out(*attention(True)),
             "a_in0": pass_first, "a_in1": pass_a_in}[only]()
            z = lax.fori_loop(0, 2, lambda i, c: c + i // 2, 0)
            acc = jnp.zeros((8, 128), U32)
            for ref in wc + (xl, xr, pq, qt, kk, vt):
                v = ref[(z,) * (len(ref.shape) - 2) + (slice(0, 16), slice(0, 128))]
                acc = acc + (v[0:8] if v.dtype == U32 else pltpu.bitcast(v, U32))
            f = xres[pl.ds(pl.multiple_of(z * 8, 8), 8), 0:128] + kvacc[z, 0:8] + zacc[:, 0:128] + zrow[z, :, 0:128]
            xin[0:16, 0:128] = _up(acc + pltpu.bitcast(f, U32))
            pltpu.sync_copy(xin.at[0:16], out_hbm.at[0:16])
            return

        with scope("a_in0"):
            pass_first()
        with scope("b_in0"):
            pass_b_in(True)
        with scope("att0"):
            attention(False)
        with scope("a_in1"):
            pass_a_in()
        with scope("b_in1"):
            pass_b_in(False)
        with scope("att1"):
            rest = attention(True)
        with scope("out"):
            pass_out(*rest)

    def run(A_x, A_wqkv, A_wo, B_x, B_wqkv, B_wo):
        any_spec = pl.BlockSpec(memory_space=pl.ANY)
        out = pl.pallas_call(
            kernel,
            out_shape=jax.ShapeDtypeStruct((S, D), BF16),
            in_specs=[any_spec] * 5,
            out_specs=any_spec,
            scratch_shapes=[
                pltpu.VMEM((S, D), BF16),
                pltpu.VMEM((D, 3 * D), BF16),
                pltpu.VMEM((D, D), BF16),
                pltpu.VMEM((D, D), BF16),
                pltpu.VMEM((D, 3 * D), BF16),
                pltpu.VMEM((D, D), BF16),
                pltpu.VMEM((S, D), F32),
                pltpu.VMEM((R, BM, BK), BF16),
                pltpu.VMEM((R, BM, BK), BF16),
                pltpu.VMEM((B, S, BK), BF16),
                pltpu.VMEM((D // 2, TM), U32),
                pltpu.VMEM((TM, D), BF16),
                pltpu.VMEM((G, 128, 128), F32),
                pltpu.VMEM((8, D), F32),
                pltpu.VMEM((B, 8, BK), F32),
                pltpu.VMEM((NT, D // 2, TM), U32),
                pltpu.VMEM((G, S // 2, 128), U32),
                pltpu.VMEM((NT, D // 2, TM), U32),
                pltpu.VMEM((UPI * DH, QB), F32),
                pltpu.VMEM((1, TM, 128), F32),
                pltpu.VMEM((1, TM, 128), F32),
                pltpu.VMEM((1, TM, BK), F32),
                pltpu.VMEM((1, DH, QB), F32),
                pltpu.VMEM((1, DH, QB), F32),
                pltpu.SemaphoreType.DMA((17,)),
                pltpu.SemaphoreType.DMA((4 * NT,)),
            ] + [pltpu.VMEM((R, BK, BK), BF16)] * 8 + [pltpu.VMEM((1, CK, QB), F32)] * (2 * NC),
            compiler_params=pltpu.CompilerParams(vmem_limit_bytes=127 * 2 ** 20, flags=flags),
            name="fused",
        )(A_x.reshape(S, D), A_wqkv, A_wo, B_wqkv, B_wo)
        return out.reshape(1, S, D)
    return run


class _Null:
    def __enter__(self):
        return None

    def __exit__(self, *a):
        return False


@jax.jit
def pallas_interleave_layers__linear_attn_block__mha_block__prompt_kernel(
    A_x: jax.Array,
    A_wqkv: jax.Array,
    A_wo: jax.Array,
    B_x: jax.Array,
    B_wqkv: jax.Array,
    B_wo: jax.Array,
):
    return make()(A_x, A_wqkv, A_wo, B_x, B_wqkv, B_wo)
```

```python
import numpy as np
import jax
import jax.numpy as jnp
from jax import lax
import jax.experimental.pallas as pl
import jax.experimental.pallas.tpu as pltpu

S, D, H, DH = 2048, 1024, 32, 32
G = D // 128
TM = 512
NT = S // TM
BM, BK = TM // 4, D // 4
R = 49
CK = 128
NC = S // CK
UPI = 8
F32, BF16, U32 = jnp.float32, jnp.bfloat16, jnp.uint32
QSCALE = float(DH ** -0.5 * np.log2(np.e))
AQ, AK, AV, AO, BQ, BKEY, BV, BO = range(8)

_LHS = (((1, 0, 1), (1, 1, 1)), ((0, 0, 1), (1, 1, 1)), ((1, 1, 1),), ((0, 0, 1), (0, 1, 1)),
        ((0, 1, 1), (1, 1, -1)), ((0, 0, 1),), ((1, 0, 1), (0, 0, -1)))
_RHS = (((0, 0, 1),), ((0, 0, 1), (1, 1, 1)), ((1, 0, 1), (0, 0, -1)), ((1, 1, 1),),
        ((1, 0, 1), (1, 1, 1)), ((0, 1, 1), (1, 1, -1)), ((0, 0, 1), (0, 1, 1)))


def _dot(a, b):
    return jnp.dot(a, b, preferred_element_type=F32)


def _pack(x):
    return pltpu.bitcast(x, U32)


def _unpack(x):
    return pltpu.bitcast(x, BF16)


def _wide(x, n):
    return lax.concatenate([x] * n, x.ndim - 1) if n > 1 else x


def _phi(t):
    return jnp.where(t > 0, t + 1.0, jnp.exp(t)) + 1e-6


def _comb(terms, get):
    out = get(*terms[0][:2])
    for i, j, sign in terms[1:]:
        out = out + get(i, j) if sign > 0 else out - get(i, j)
    return out


def _operands(table, k, quadrant):
    q = _comb(table[k], quadrant)
    q = [[q[a:a + 1, :, b * BK:(b + 1) * BK] for b in range(2)] for a in range(2)]
    return [_comb(t, lambda a, b: q[a][b]) for t in table]


def _strassen(prod, levels, emit, base=0):
    if levels == 0:
        return [lambda: emit(0, 0, prod(base))]
    n, h = 7 ** (levels - 1), 2 ** (levels - 1)
    held = {}

    def step(k):
        def take(i, j, v):
            m = held.setdefault((i, j), {})
            if k == 2:
                emit(h + i, j, m[0] + v)
                v = m[1] + v
            elif k == 3:
                m[2] = m[2] - v
            elif k == 4:
                emit(i, j, m[2] + v)
            elif k == 5:
                emit(i, h + j, m[3] + v)
                v = (m[1] + v) - m[0]
            elif k == 6:
                emit(h + i, h + j, m[5] + v)
            m[k] = v
        return take
    return [t for k in range(7) for t in _strassen(prod, levels - 1, step(k), base + k * n)]


def _swap_blocks(t):
    lane = lax.broadcasted_iota(jnp.int32, t[0].shape, 1)
    for bit, sh in ((1, 8), (2, 16)):
        low = (lane & sh) == 0
        t = [jnp.where(low, pltpu.roll(t[b ^ bit], 128 - sh, 1), t[b]) if b & bit
             else jnp.where(low, t[b], pltpu.roll(t[b ^ bit], sh, 1)) for b in range(4)]
    return t


class _Task:
    def __init__(self, run, keys=()):
        self.run, self.keys = run, keys


def _weave(main, side=(), lo=0.0, hi=1.0):
    last = {key: n for n, t in enumerate(side) for key in t.keys}
    k = 0
    for n, t in enumerate(main):
        must = max([last.get(key, -1) for u in main[n:n + 3] for key in u.keys], default=-1)
        while k < len(side) and (k <= must or (lo + (hi - lo) * k / len(side)) * len(main) < n + 1):
            side[k].run()
            k += 1
        t.run()
    for t in side[k:]:
        t.run()


TUNE = dict(
    first=dict(lag=3, due=6, n0=28, k0=3, rest=0.6),
    second=dict(lag=4, due=5, n1=6, n2=35, rest=0.78, lo=0.05, hi=0.6),
    last=dict(lag=4, due=4, n1=5, n2=26, rest=0.75, den=12, hi=0.75, nq=9, fold=0.8, tdue=6),
    soft=dict(lag=4, due=3, n1=6, n2=40, rest=0.75, den=20, hi=0.7),
    soft_last=dict(lag=4, due=3, rest=0.82),
    tail=dict(lag=3, due=3, at=50),
    out=dict(lag=2, due=0),
)
SR, PR = 32, 64


def _kernel(x_hbm, wa_hbm, woa_hbm, wb_hbm, wob_hbm, out_hbm,
            xio, wa, woa, wb, wtmp, mtmp, xres, xl, xr, qo, pkt, vb, kvacc, sums, zrow,
            qt, kk, vt, ot, mu, rs, rden, acc0, acc1, sem_in, sem_out, *bufs):
    wc, sbuf = bufs[:8], bufs[8:]

    zs, never, ticks, owed, cfg = [], {}, [], [], {}

    def enter(i):
        zs[:] = [i >> (8 + k) for k in range(8)]
        never.clear()
        ticks.clear()
        owed.clear()

    def loop(n, fn):
        def body(i, _):
            enter(i)
            fn(i)
            return i
        enter(lax.fori_loop(0, n, body, 0))

    def after(dep, v):
        if v.shape not in never:
            never[v.shape] = jnp.broadcast_to(zs[6], v.shape) != 0
        return lax.select(never[v.shape], dep, v)

    def paced(v):
        if len(ticks) < cfg["lag"]:
            return v
        flat = v.reshape(-1, 8, v.shape[-1])
        dep = jnp.broadcast_to(_wide(ticks[-cfg["lag"]], v.shape[-1] // 128), flat.shape)
        return after(dep, flat).reshape(v.shape)

    def put(dst, table, k, r0, quadrant):
        ts = _operands(table, k, quadrant)
        dst[7 * k:7 * k + 7, pl.ds(r0, 8), :] = lax.concatenate(ts, 0).astype(BF16)
        return ts

    def operand_tasks(dst, key, table, ks, quadrant):
        def task(k, r0):
            def run():
                ts = put(dst, table, k, r0, lambda i, j: quadrant(k, r0, i, j))
                if cfg["due"]:
                    t = (ts[0] + ts[3] if table is _LHS else ts[4] + ts[6])[0]
                    owed.append((len(ticks) + cfg["due"], t[:, :128] + t[:, 128:]))
            return _Task(run, ((key, k),))
        return [task(k, r0) for k in ks for r0 in range(0, dst.shape[1], 8)]

    def burst(dst, table, quadrant, lo, hi, unroll):
        def body(n):
            for h in range(unroll):
                r0 = pl.multiple_of(lo + (n * unroll + h) * 8, 8)
                q = [[quadrant(r0, i, j) for j in range(2)] for i in range(2)]
                for k in range(7):
                    put(dst, table, k, r0, lambda i, j: q[i][j])
        loop((hi - lo) // (8 * unroll), body)

    def read(ref, a0, r0, i, j, c0=0):
        return ref[pl.ds(a0 + 2 * i, 2), pl.ds(r0, 8), pl.ds(c0 + 2 * j * BK, 2 * BK)].astype(F32)

    def plain_ops(dst, key, table, ks, ref, a0, c0=0):
        a0 = [a0 + z for z in zs]

        def quadrant(k, r0, i, j):
            v = read(ref, a0[k], r0, i, j, c0)
            return paced(v) if (i, j) == table[k][0][:2] else v
        return operand_tasks(dst, key, table, ks, quadrant)

    def w_burst(u, ref, c0, lo=0, hi=BK):
        burst(wc[u], _RHS, lambda r0, i, j: read(ref, 0, r0, i, j, c0), lo, hi, 4)

    def ln_stats(src, t, blocks=range(4)):
        def mean(a, rr):
            x = src[4 * t + a, rr, :].astype(F32)
            v = paced(x[:, :128])
            for g in range(1, G):
                v = v + x[:, g * 128:(g + 1) * 128]
            mu[a, rr, :] = jnp.broadcast_to(jnp.sum(v, axis=-1, keepdims=True) * (1.0 / D), (SR, 128))

        def rstd(a, rr):
            x = src[4 * t + a + zs[7], rr, :].astype(F32) - _wide(paced(mu[a + zs[7], rr, :]), G)
            rs[a, rr, :] = jnp.broadcast_to(
                lax.rsqrt(jnp.mean(x * x, axis=-1, keepdims=True) + 1e-5), (SR, 128))
        return [[_Task(lambda f=f, a=a, r0=r0: f(a, slice(r0, r0 + SR)))
                 for a in blocks for r0 in range(0, BM, SR)] for f in (mean, rstd)]

    def normed(src, a0, z, r0, i, j):
        idx = (pl.ds(z + 2 * i, 2), pl.ds(r0, 8))
        return (read(src, a0, r0, i, j) - _wide(paced(mu[idx]), 4)) * _wide(rs[idx], 4)

    def ln_ops(src, t, ks, col_sums):
        a0 = [4 * t + z for z in zs]

        def quadrant(k, r0, i, j):
            v = normed(src, a0[k], zs[k], r0, i, j)
            if col_sums and k in (4, 6):
                sums[2, :, 2 * j * BK:(2 * j + 2) * BK] += v[0] + v[1]
            return v
        return operand_tasks(xl, "xl", _LHS, ks, quadrant)

    def ln_head(main, src, t):
        means, rstds = ln_stats(src, t)
        n1, n2 = cfg["n1"], cfg["n2"]
        assert n2 >= 7
        _weave(main[:n1], means, 2 / n1)
        _weave(main[n1:n2], rstds, 0.05)
        _weave(main[n2:], ln_ops(src, t, range(1), False), 3 / (len(main) - n2), 0.93)

    def ln_rest(main, src, t, col_sums):
        _weave(main, ln_ops(src, t, range(1, 7), col_sums), 0.0, cfg["rest"])

    def project(lhs, key, u, emit):
        def prod(r):
            w = wc[u][r]
            if owed and owed[0][0] <= len(ticks):
                w = _pack(w)
                top = w[:8, :128]
                while owed and owed[0][0] <= len(ticks):
                    top = after(pltpu.bitcast(owed.pop(0)[1], U32), top)
                w = _unpack(lax.concatenate([lax.concatenate([top, w[:8, 128:]], 1), w[8:]], 0))
            v = _dot(lhs[r], w)
            ticks.append(v[:8, :128])
            return v
        thunks = _strassen(prod, 2, lambda bi, bj, v: emit(bi, slice(bj * BK, (bj + 1) * BK), bj, v))
        return [_Task(t, ((key, r // 7), (u, r // 7))) for r, t in enumerate(thunks)]

    def transposed(ref, idx, bi, bj, v, due=0):
        v = _pack(v.astype(BF16).T)
        ref[idx + (pl.ds(bj * (BK // 2), BK // 2), pl.ds(bi * BM, BM))] = v
        if due:
            owed.append((len(ticks) + due, v[56:64] | v[120:]))

    def residual(src, t, u):
        def emit(bi, cs, bj, v):
            xres[4 * t + bi, :, cs] = src[4 * t + bi, :, cs].astype(F32) + v
        return project(xr, "xr", u, emit)

    def out_copy(t, i, j):
        idx = (pl.ds(4 * t + 2 * i, 2), slice(None), pl.ds(2 * j * BK, 2 * BK))
        return pltpu.make_async_copy(xio.at[idx], out_hbm.at[idx], sem_out)

    def output(t, lhs, key):
        def emit(bi, cs, bj, v):
            xio[4 * t + bi, :, cs] = (xres[4 * t + bi, :, cs] + v).astype(BF16)
            if bi % 2 and bj % 2:
                out_copy(t, bi // 2, bj // 2).start()
        return project(lhs, key, BO, emit)

    def lin_qkv(t, due=0):
        def emit_k(bi, cs, bj, v):
            v = _phi(v)
            sums[0, :, cs] += jnp.sum(v.reshape(BM // 8, 8, BK), axis=0)
            transposed(pkt, (), bi, bj, v, due)

        def emit_v(bi, cs, bj, v):
            sums[1, :, cs] += jnp.sum(v.reshape(BM // 8, 8, BK), axis=0)
            vb[bi * BM:(bi + 1) * BM, cs] = v.astype(BF16)

        def emit_q(bi, cs, bj, v):
            qo[4 * t + bi, :, cs] = _phi(v).astype(BF16)

        def kv(g):
            kvacc[g] += _dot(_unpack(pkt[g * 64:(g + 1) * 64, :]), vb[:, g * 128:(g + 1) * 128])
        return (project(xl, "xl", AK, emit_k), project(xl, "xl", AV, emit_v),
                project(xl, "xl", AQ, emit_q), [_Task(lambda g=g: kv(g)) for g in range(G)])

    def lin_reset():
        kvacc[...] = jnp.zeros(kvacc.shape, F32)
        sums[...] = jnp.zeros(sums.shape, F32)

    def lanes(b, j):
        return slice(b * BK + j * 128, b * BK + j * 128 + 128)

    def permute_wq(a, r0, j):
        t = _swap_blocks([paced(pltpu.bitcast(wa[a, r0:r0 + PR, lanes(b, j)], F32)) for b in range(4)])
        for b in range(4):
            wtmp[a, r0:r0 + PR, lanes(b, j)] = _unpack(t[b])

    def col_sum(n, cs=slice(None)):
        return jnp.sum(sums[n, :, cs], axis=0, keepdims=True)

    def lin_z():
        for j in range(2):
            t = _swap_blocks([jnp.broadcast_to(col_sum(0, lanes(b, j)), (8, 128)) for b in range(4)])
            for b in range(4):
                zrow[0, :, lanes(b, j)] = t[b]

    def lin_fold():
        xs, drift = [], {}

        def v_sum(g, h):
            if not xs:
                x = jnp.broadcast_to(col_sum(2), (8, D))
                hi = x.astype(BF16).astype(F32)
                xs.append(lax.concatenate([hi, x - hi], 0).astype(BF16))
            w = wa[2 * h:2 * h + 2, :, 2 * D + g * 128:2 * D + (g + 1) * 128].reshape(2 * BK, 128)
            c = _dot(xs[0][:, 2 * h * BK:(2 * h + 2) * BK], w)
            drift[g] = drift.get(g, 0.0) + (c[0:1] + c[8:9])

        def fold(g, n):
            kv, gs = kvacc[g], slice(g * 128, (g + 1) * 128)
            kv = kv * jnp.broadcast_to(1.0 / col_sum(0, gs), (128, 128)).T
            kv = kv + (drift[g] - col_sum(1, gs)) * (1.0 / S)
            same = (lax.broadcasted_iota(jnp.int32, (128, 128), 0) // DH
                    == lax.broadcasted_iota(jnp.int32, (128, 128), 1) // DH)
            cs = slice(n * 512, (n + 1) * 512)
            m = _dot(jnp.where(same, kv, 0.0).astype(BF16), woa[gs, cs]).reshape(4, 4, 8, 512)
            hb, j = divmod(g, 2)
            for h in range(4):
                r0 = j * 128 + h * DH + hb * 8
                mtmp[:, r0:r0 + 8, cs] = m[h]
        return ([_Task(lambda g=g, h=h: v_sum(g, h)) for g in range(G) for h in range(2)],
                [_Task(lambda g=g, n=n: fold(g, n)) for n in range(2) for g in range(G)])

    def lin_ops(main, t):
        def den(a, rr):
            v = qo[4 * t + a, rr, :].astype(F32).reshape(SR // 8, 8, D) * paced(zrow[pl.ds(zs[7], 1)])
            v = v[:, :, :2 * BK] + v[:, :, 2 * BK:]
            v = (v[:, :, :BK] + v[:, :, BK:]).reshape(SR, BK)
            v = lax.concatenate([v[:, :128], v[:, 128:]], 0)
            lane = lax.broadcasted_iota(jnp.int32, v.shape, 1)
            for sh in (1, 2, 4):
                v = v + jnp.where((lane & sh) != 0, pltpu.roll(v, sh, 1), pltpu.roll(v, 128 - sh, 1))
            v = 1.0 / (v + 1e-6)
            rden[a, rr, :] = lax.concatenate([v[:SR], v[SR:]], 1)
        a0 = [4 * t + z for z in zs]

        def quadrant(k, r0, i, j):
            v = read(qo, a0[k], r0, i, j) * _wide(paced(rden[pl.ds(zs[k] + 2 * i, 2), pl.ds(r0, 8)]), 2)
            return v * zrow[pl.ds(zs[r0 // 8 % 8], 1), :, 2 * j * BK:(2 * j + 2) * BK]
        ns = cfg["den"]
        _weave(main[:ns + 5], [_Task(lambda a=a, r0=r0: den(a, slice(r0, r0 + SR)))
                               for a in range(4) for r0 in range(0, BM, SR)], 0.0, ns / (ns + 5))
        _weave(main[ns + 5:], operand_tasks(xr, "xr", _LHS, range(7), quadrant), 0.0, cfg["hi"])

    def lin_last(src, keys):
        cfg.update(TUNE["last"])
        nq = cfg["nq"]
        k, v, q, kv = lin_qkv(NT - 1, cfg["tdue"])
        v_sum, fold = lin_fold()
        if keys:
            ln_rest(k, src, NT - 1, True)
        _weave(v[:2])
        lin_z()
        for n, t in enumerate(v_sum):
            v.insert(24 + 2 * n, t)
        lin_ops(v[2:] + q[:2] + kv + q[2:4] + fold, 0)
        _weave(q[4:nq] + residual(src, 0, AO), plain_ops(wc[AO], AO, _RHS, range(7), mtmp, 0), 0.02, cfg["fold"])
        ln_head(q[nq:], xres, 0)

    def att_qkv(t):
        def emit_k(bi, cs, bj, v):
            v = _pack(v.astype(BF16))
            for j in range(2):
                kk[2 * bj + j, 4 * t + bi] = v[:, j * 128:(j + 1) * 128]
        return (project(xl, "xl", BQ, lambda bi, cs, bj, v: transposed(qt, (t,), bi, bj, v * QSCALE)),
                project(xl, "xl", BV, lambda bi, cs, bj, v: transposed(vt, (t,), bi, bj, v)),
                project(xl, "xl", BKEY, emit_k))

    def attention(tail, tail_matmuls):
        lead, steps = NC + 1, UPI * NC
        iters = NT * H // UPI

        def units(it):
            heads = [it * UPI + u for u in range(UPI + 2)]
            return [(h // H, h % H // 4, pl.ds(pl.multiple_of(h % H * (DH // 2), DH // 2), DH // 2))
                    for h in heads]

        def scores(unit, u, c, m):
            qb, g, hs = unit
            parts = [jnp.zeros((DH // 2, TM), U32)] * 4
            parts[u % 4] = qt[qb, hs, :]
            s = _dot(_unpack(kk[g, c]), _unpack(lax.concatenate(parts, 0)))
            sbuf[u % 2 * NC + c][0] = s
            mc = jnp.max(s.reshape(CK // 8, 8, TM), axis=0)
            m = mc if c == 0 else jnp.maximum(m, mc)
            return jnp.broadcast_to(jnp.max(m, axis=0, keepdims=True), (8, TM)) if c == NC - 1 else m

        def flush(it, n):
            cs = pl.ds(pl.multiple_of(it % (H // UPI) * (UPI * DH), UPI * DH), UPI * DH)
            qo[it // (H // UPI) * 4 + n, :, cs] = ot[:, n * BM:(n + 1) * BM].astype(BF16).T

        def block(it, m_cur, m_run, extra=None):
            us, maxes, accs, l = units(it), [m_cur], [], None
            for t in range(steps):
                u, c = divmod(t, NC)
                s = sbuf[u % 2 * NC + c][zs[0]]
                ua, ca = divmod(t + lead, NC)
                more = extra is None or ua < UPI
                if more:
                    m_run = scores(us[ua], ua, ca, m_run)
                    if ca == NC - 1:
                        maxes.append(m_run)
                if t in (4, 6, 8, 10):
                    flush(jnp.maximum(it - 1, 0), t // 2 - 2)
                if extra is not None:
                    extra(t)
                m = maxes[u]
                if t > 0:
                    m = lax.select(l < 0, accs[-2][:8] if t > 1 and (more or tail_matmuls) else l, m)
                p = jnp.exp2(s.reshape(CK // 8, 8, TM) - m[None])
                pairs = p.reshape(CK // 16, 16, TM)
                pairs = (pairs[:, :8] + pairs[:, 8:]).reshape(CK // 2, TM)
                for r in reversed(range(0, CK // 2, 8)):
                    l = pairs[r:r + 8] if c == 0 and r == CK // 2 - 8 else l + pairs[r:r + 8]
                v = _unpack(vt[c // 4, us[u][2], c % 4 * CK:(c % 4 + 1) * CK])
                acc = _dot(v, p.reshape(CK, TM).astype(BF16))
                if c > 0:
                    acc = (acc0, acc1)[c % 2][zs[0]] + acc
                if c < NC - 1:
                    (acc1, acc0)[c % 2][0] = acc
                else:
                    ot[u * DH:(u + 1) * DH, :] = acc * pltpu.reciprocal(
                        jnp.sum(l, axis=0, keepdims=True), full_range=False)
                accs.append(acc)
                ticks.append(acc[:8, :128])
            return maxes[-1], m_run

        ot[...] = jnp.zeros(ot.shape, F32)
        m = [None]
        for t in range(lead):
            m.append(scores(units(0)[t // NC], t // NC, t % NC, m[-1]))

        def body(it, carry):
            enter(it)
            return block(it, *carry[:2]) + (it,)
        m_cur, m_run, it = lax.fori_loop(0, iters - 1, body, (m[-2], m[-1], 0))
        enter(it)
        block(iters - 1, m_cur, m_run, tail(steps - lead))
        for n in range(4):
            flush(iters - 1, n)

    def o_ops(t, dst=xr, key="xr"):
        return plain_ops(dst, key, _LHS, range(7), qo, 4 * t)

    def first_linear():
        cfg.update(TUNE["first"])
        full, n0, k0 = slice(None), cfg["n0"], cfg["k0"]
        jobs = [(x_hbm, xio, (slice(0, 2),)), (x_hbm, xio, (slice(2, 4),)),
                (wa_hbm, wa, (full, slice(0, BK // 2), slice(D, 2 * D))),
                (wa_hbm, wa, (full, slice(BK // 2, BK), slice(D, 2 * D))),
                (wa_hbm, wa, (full, full, slice(2 * D, 3 * D))), (wa_hbm, wa, (full, full, slice(0, D))),
                (x_hbm, xio, (slice(4, 8),)), (x_hbm, xio, (slice(8, 16),)),
                (wb_hbm, wb, (full,)), (woa_hbm, woa, (full,))]
        cps = [pltpu.make_async_copy(a.at[idx], b.at[idx], sem_in.at[n]) for n, (a, b, idx) in enumerate(jobs)]
        cps.append(pltpu.make_async_copy(wob_hbm, wa.at[:, :, D:2 * D], sem_in.at[10]))
        for c in cps[:4]:
            c.start()
        lin_reset()
        zs[:] = [0] * 8
        for n in range(2):
            cps[n].wait()
            _weave([], sum(ln_stats(xio, 0, (2 * n, 2 * n + 1)), []))

        def quadrant(r0, i, j):
            v = normed(xio, 0, 0, r0, i, j)
            sums[2, :, 2 * j * BK:(2 * j + 2) * BK] += v[0] + v[1]
            return v
        burst(xl, _LHS, quadrant, 0, BM, 1)
        cps[2].wait()
        w_burst(AK, wa, D, 0, BK // 2)
        cps[4].start()
        cps[5].start()
        cps[3].wait()
        w_burst(AK, wa, D, BK // 2, BK)
        _weave(lin_qkv(0)[0])
        cps[4].wait()
        w_burst(AV, wa, 2 * D)
        cps[5].wait()
        cps[6].start()

        def tile(t):
            k, v, q, kv = lin_qkv(t)
            assert n0 >= 7 * k0
            _weave(v, [_Task(lambda a=a, r0=r0, j=j: permute_wq(a, r0, j))
                       for a in range(4) for r0 in range(0, BK, PR) for j in range(2)], 0.0, 0.9)

            @pl.when(t == 0)
            def _():
                cps[6].wait()
                for c in cps[7:]:
                    c.start()
                w_burst(AQ, wtmp, 0)

            @pl.when(t == 1)
            def _():
                cps[7].wait()

            @pl.when(t == 2)
            def _():
                for c in cps[8:]:
                    c.wait()
                for n in range(3):
                    w_burst(BQ + n, wb, n * D)
            enter(t)
            means, rstds = ln_stats(xio, t + 1)
            _weave(kv, means)
            _weave(q[:n0], rstds, 0.05)
            _weave(q[n0:], ln_ops(xio, t + 1, range(k0), True), 0.1)
            _weave(k, ln_ops(xio, t + 1, range(k0, 7), True), 0.0, cfg["rest"])
        loop(NT - 1, tile)
        lin_last(xio, False)

    def second_linear():
        def tile(t):
            k, v, q, kv = lin_qkv(t)
            ln_rest(k, xres, t, True)
            _weave(v + residual(xres, t + 1, BO), o_ops(t + 1), cfg["lo"], cfg["hi"])
            ln_head(q + kv, xres, t + 1)
        cfg.update(TUNE["second"])
        lin_reset()
        loop(NT - 1, tile)
        lin_last(xres, True)

    def softmax_inputs(first):
        def tile(t):
            q, v, k = att_qkv(t)
            ln_rest(q, xres, t, False)
            lin_ops(v + residual(xio if first else xres, t + 1, AO), t + 1)
            ln_head(k, xres, t + 1)
        cfg.update(TUNE["soft"])
        loop(NT - 1, tile)
        cfg.update(TUNE["soft_last"])
        q, v, k = att_qkv(NT - 1)
        ln_rest(q, xres, NT - 1, False)
        _weave(v + k, plain_ops(wc[BO], BO, _RHS, range(7), wa, 0, D) if first else [], 0.0, 0.97)

    def first_softmax():
        cfg.update(TUNE["tail"])
        t_op = cfg["at"]

        def tail(end):
            side = o_ops(0)
            means, rstds = ln_stats(xres, 0)
            ln = means + rstds + [_Task(lambda: None)] * 3 + ln_ops(xres, 0, range(1), False)

            def extra(t):
                if 12 < t < t_op and side:
                    side.pop(0).run()
                if t == t_op:
                    _weave(residual(xres, 0, BO), side, 0.0, 0.8)
                if t > t_op + 1 and ln:
                    ln.pop(0).run()
                assert t < UPI * NC - 1 or not ln
            return extra
        attention(tail, False)

    def second_softmax():
        main = output(0, xr, "xr")
        cfg.update(TUNE["out"])

        def tail(end):
            side = o_ops(0)

            def extra(t):
                for _ in range(2 if t > 16 else 0):
                    if side:
                        side.pop(0).run()
                if t >= end:
                    main.pop(0).run()
            return extra
        attention(tail, True)
        slots = ((xr, "xr"), (xl, "xl"))
        for t in range(NT):
            _weave(main if t == 0 else output(t, *slots[t % 2]),
                   o_ops(t + 1, *slots[1 - t % 2]) if t + 1 < NT else [], 0.0, 0.97)
        for t in range(NT):
            for q in range(4):
                out_copy(t, q // 2, q % 2).wait()

    first_linear()
    softmax_inputs(True)
    first_softmax()
    second_linear()
    softmax_inputs(False)
    second_softmax()


@jax.jit
def pallas_interleave_layers__linear_attn_block__mha_block__prompt_kernel(
    A_x: jax.Array,
    A_wqkv: jax.Array,
    A_wo: jax.Array,
    B_x: jax.Array,
    B_wqkv: jax.Array,
    B_wo: jax.Array,
):
    del B_x
    hbm = pl.BlockSpec(memory_space=pl.ANY)
    out = pl.pallas_call(
        _kernel,
        out_shape=jax.ShapeDtypeStruct((4 * NT, BM, D), BF16),
        in_specs=[hbm] * 5,
        out_specs=hbm,
        scratch_shapes=[
            pltpu.VMEM((4 * NT, BM, D), BF16),
            pltpu.VMEM((4, BK, 3 * D), BF16),
            pltpu.VMEM((D, D), BF16),
            pltpu.VMEM((4, BK, 3 * D), BF16),
            pltpu.VMEM((4, BK, D), BF16),
            pltpu.VMEM((4, BK, D), F32),
            pltpu.VMEM((4 * NT, BM, D), F32),
            pltpu.VMEM((R, BM, BK), BF16),
            pltpu.VMEM((R, BM, BK), BF16),
            pltpu.VMEM((4 * NT, BM, D), BF16),
            pltpu.VMEM((D // 2, TM), U32),
            pltpu.VMEM((TM, D), BF16),
            pltpu.VMEM((G, 128, 128), F32),
            pltpu.VMEM((3, 8, D), F32),
            pltpu.VMEM((1, 8, D), F32),
            pltpu.VMEM((NT, D // 2, TM), U32),
            pltpu.VMEM((G, NC, CK // 2, 128), U32),
            pltpu.VMEM((NT, D // 2, TM), U32),
            pltpu.VMEM((UPI * DH, TM), F32),
            pltpu.VMEM((4, BM, 128), F32),
            pltpu.VMEM((4, BM, 128), F32),
            pltpu.VMEM((4, BM, BK), F32),
            pltpu.VMEM((1, DH, TM), F32),
            pltpu.VMEM((1, DH, TM), F32),
            pltpu.SemaphoreType.DMA((11,)),
            pltpu.SemaphoreType.DMA(()),
        ] + [pltpu.VMEM((R, BK, BK), BF16)] * 8 + [pltpu.VMEM((1, CK, TM), F32)] * (2 * NC),
        compiler_params=pltpu.CompilerParams(vmem_limit_bytes=126 * 2 ** 20),
        name="interleaved_attention",
    )(A_x.reshape(4 * NT, BM, D), A_wqkv.reshape(4, BK, 3 * D), A_wo,
      B_wqkv.reshape(4, BK, 3 * D), B_wo.reshape(4, BK, D))
    return out.reshape(1, S, D)
```
